```python
import jax
import jax.numpy as jnp

def _softmax(x, axis=-1):
    return jax.nn.softmax(x, axis=axis)
def _gelu(x):
    return jax.nn.gelu(x, approximate=True)
def _silu(x):
    return jax.nn.silu(x)
def _sigmoid(x):
    return jax.nn.sigmoid(x)
def _layernorm(x, axis=-1, eps=1e-5):
    m = jnp.mean(x, axis=axis, keepdims=True)
    v = jnp.var(x, axis=axis, keepdims=True)
    return (x - m) / jnp.sqrt(v + eps)
def _scatter_add(tgt, idx, src, axis=0):
    return tgt.at[idx].add(src)
def _segment_sum(src, seg, n):
    return jax.ops.segment_sum(src, seg, n)
class _Rng:
    def __init__(self, key):
        self._k = key
    def _next(self):
        self._k, sub = jax.random.split(self._k)
        return sub
    def normal(self, shape):
        return jax.random.normal(self._next(), shape, dtype=jnp.bfloat16)
    def randint(self, lo, hi, shape):
        return jax.random.randint(self._next(), shape, lo, hi, dtype=jnp.int32)
    def uniform(self, shape, lo=0.0, hi=1.0):
        return jax.random.uniform(self._next(), shape, jnp.bfloat16, lo, hi)
    def permutation(self, n):
        return jax.random.permutation(self._next(), n)


kernel_name = 'standalone__batchnorm__sampling'

def setup_inputs():
    _rng = _Rng(jax.random.key(int.from_bytes(__import__("os").urandom(4), "little")))
    _w = (lambda a: (lambda t: t.astype(jnp.bfloat16) if jnp.issubdtype(t.dtype, jnp.floating) else t)(jnp.asarray(a)))
    B, S, C = 1024, 32, 576
    K = 3
    return {
        "x": _w((lambda *s: _rng.normal(s) * 0.05)(B, S, C)),
        "w": _w((lambda *s: _rng.normal(s) * 0.05)(K, C, C) * (1.0 / (K * C) ** 0.5)),
        "mean": _w((lambda *s: _rng.normal(s) * 0.05)(C) * 0.1),
        "var": _w(jnp.abs((lambda *s: _rng.normal(s) * 0.05)(C)) + 0.5),
        "g": _w((lambda *s: _rng.normal(s) * 0.05)(C) + 1.0),
        "b": _w((lambda *s: _rng.normal(s) * 0.05)(C) * 0.1),
    }

def reference(x, w, mean, var, g, b):
    K = 3
    P = K // 2
    S = x.shape[1]
    xp = jnp.pad(x, ((0, 0), (P, P), (0, 0)))
    y = sum(jnp.einsum('bsc,cd->bsd', xp[:, k:k + S, :], w[k]) for k in range(K))
    inv_std = 1.0 / jnp.sqrt(var + 1e-5)
    y = (y - mean) * (g * inv_std) + b
    return _silu(y)
```

```python
import jax
import jax.numpy as jnp
import jax.experimental.pallas as pl
import jax.experimental.pallas.tpu as pltpu

f32 = jnp.float32
bf16 = jnp.bfloat16
BN = 128


def _kernel(xm_ref, xc_ref, xp_ref, w_ref, mean_ref, var_ref, g_ref, b_ref, o_ref, u_ref, bias_ref):
    t = pl.program_id(0)
    nt = pl.num_programs(0)
    C = xc_ref.shape[1]

    @pl.when(jnp.logical_and(t == 0, pl.program_id(1) == 0))
    def _():
        sc = g_ref[...].astype(f32) * jax.lax.rsqrt(var_ref[...].astype(f32) + 1e-5)
        bias = b_ref[...].astype(f32) - mean_ref[...].astype(f32) * sc
        sc = 0.5 * sc
        bias = 0.5 * bias
        bias_ref[...] = jnp.transpose(jnp.broadcast_to(bias, (128, C)))
        scT = jnp.transpose(jnp.broadcast_to(sc, (128, C)))[:, 0:1]
        g0 = jnp.transpose(w_ref[0].astype(f32)) * scT
        g1 = jnp.transpose(w_ref[1].astype(f32)) * scT
        g2 = jnp.transpose(w_ref[2].astype(f32)) * scT
        u_ref[0] = (g0 * 0.25).astype(bf16)
        u_ref[1] = ((g0 + g1 + g2) * (-1.0 / 6)).astype(bf16)
        u_ref[2] = ((g0 - g1 + g2) * (-1.0 / 6)).astype(bf16)
        u_ref[3] = (g0 * (1.0 / 24) + g1 * (1.0 / 12) + g2 * (1.0 / 6)).astype(bf16)
        u_ref[4] = (g0 * (1.0 / 24) - g1 * (1.0 / 12) + g2 * (1.0 / 6)).astype(bf16)
        u_ref[5] = g2.astype(bf16)

    d0 = jnp.where(t == 0, 0.0, xm_ref[0].astype(f32))
    d1 = xc_ref[0].astype(f32)
    d2 = xc_ref[1].astype(f32)
    d3 = xc_ref[2].astype(f32)
    d4 = xc_ref[3].astype(f32)
    d5 = jnp.where(t == nt - 1, 0.0, xp_ref[0].astype(f32))
    a = d4 - 4.0 * d2
    b = d3 - 4.0 * d1
    c = d4 - d2
    e = 2.0 * (d3 - d1)
    v0 = (4.0 * (d0 - d2) + c).astype(bf16)
    v1 = (a + b).astype(bf16)
    v2 = (a - b).astype(bf16)
    v3 = (c + e).astype(bf16)
    v4 = (c - e).astype(bf16)
    v5 = (4.0 * (d1 - d3) + (d5 - d3)).astype(bf16)
    dot = lambda i, v: jnp.dot(u_ref[i], v, preferred_element_type=f32)
    m0, m1, m2, m3, m4, m5 = (dot(i, v) for i, v in enumerate((v0, v1, v2, v3, v4, v5)))
    m1 = m1 + jnp.tile(bias_ref[...], (1, BN // 128))
    s1 = m1 + m2
    dd1 = m1 - m2
    s2 = m3 + m4
    dd2 = m3 - m4
    ys = [m0 + s1 + s2, dd1 + 2.0 * dd2, s1 + 4.0 * s2, dd1 + 8.0 * dd2 + m5]
    for j in range(4):
        h = ys[j]
        o_ref[j] = (h * jnp.tanh(h) + h).astype(o_ref.dtype)


@jax.jit
def pallas_standalone__batchnorm__sampling_kernel(x, w, mean, var, g, b):
    B, S, C = x.shape
    xt = jnp.transpose(x, (1, 2, 0))
    vec = pl.BlockSpec((1, C), lambda t, i: (0, 0))
    NT = S // 4
    out = pl.pallas_call(
        _kernel,
        grid=(NT, B // BN),
        in_specs=[pl.BlockSpec((1, C, BN), lambda t, i: (jnp.maximum(4 * t - 1, 0), 0, i)),
                  pl.BlockSpec((4, C, BN), lambda t, i: (t, 0, i)),
                  pl.BlockSpec((1, C, BN), lambda t, i: (jnp.minimum(4 * t + 4, S - 1), 0, i)),
                  pl.BlockSpec((3, C, C), lambda t, i: (0, 0, 0)),
                  vec, vec, vec, vec],
        out_specs=pl.BlockSpec((4, C, BN), lambda t, i: (t, 0, i)),
        out_shape=jax.ShapeDtypeStruct((S, C, B), x.dtype),
        scratch_shapes=[pltpu.VMEM((6, C, C), bf16), pltpu.VMEM((C, 128), f32)],
        compiler_params=pltpu.CompilerParams(dimension_semantics=("arbitrary", "arbitrary"),
                                             vmem_limit_bytes=100 * 2**20),
    )(xt, xt, xt, w, mean.reshape(1, C), var.reshape(1, C), g.reshape(1, C), b.reshape(1, C))
    return jnp.transpose(out, (2, 0, 1))
```

```python
import jax, jax.numpy as jnp
import jax.experimental.pallas as pl
import jax.experimental.pallas.tpu as pltpu
f32 = jnp.float32; bf16 = jnp.bfloat16; i32 = jnp.int32

def _make(BN=128, vmem=100, flags=None, KP=640, NB=4, PU=4, X0=1):
    def kernel(x_hbm, w_hbm, mean_ref, var_ref, g_ref, b_ref, o_hbm,
               xs, w_ref, wsem, u_ref, bias_ref, sc_ref, wt_ref, xsem, osem, *ob):
        S, C, B = x_hbm.shape
        NT = S // 4
        NU = NT * (B // BN)
        NBLK = NU // NB
        C2 = C // 2
        TB = NT // NB

        NSEM = 2 * NB + 1
        def x_copy(q):
            b, t = q // NT, q % NT
            return pltpu.make_async_copy(
                x_hbm.at[pl.ds(4 * t, 4), :, pl.ds(pl.multiple_of(b * BN, BN), BN)],
                xs.at[b % 2, pl.ds(4 * t + 1, 4)], xsem.at[q % NSEM])

        def o_copy(q, n, slot):
            b, t = q // NT, q % NT
            return pltpu.make_async_copy(
                ob[n].at[slot], o_hbm.at[pl.ds(4 * t, 4), :, pl.ds(pl.multiple_of(b * BN, BN), BN)], osem.at[slot, n])

        wcp = pltpu.make_async_copy(w_hbm, w_ref, wsem)
        wcp.start()
        for q in range(X0):
            x_copy(q).start()
        zrow = jnp.zeros((C, BN), bf16)
        for s in range(2):
            xs[s, 0] = zrow
            xs[s, S + 1] = zrow

        row = lambda r: r[...].astype(f32).reshape(1, C)
        sc = row(g_ref) * jax.lax.rsqrt(row(var_ref) + 1e-5)
        bias = row(b_ref) - row(mean_ref) * sc
        sc = 0.5 * sc
        bias = 0.5 * bias
        bias_ref[...] = jnp.transpose(jnp.broadcast_to(bias, (128, C)))
        scT = jnp.transpose(jnp.broadcast_to(sc, (128, C)))
        sc_ref[...] = scT
        wcp.wait()
        for q in range(X0, NB + 1):
            x_copy(q).start()
        for k in range(3):
            wk = jnp.concatenate([w_ref[k], jnp.zeros((KP - C, C), bf16)], axis=0)
            wt_ref[k] = pltpu.bitcast(jnp.transpose(wk), i32)

        def prep(r, carry):
            r8 = pl.multiple_of(r * 8, 8)
            ws = [wt_ref[k, pl.ds(r8, 8), :] for k in range(3)]
            res = []
            for half in range(2):
                sT = jnp.tile(sc_ref[pl.ds(r * 16 + half, 8, stride=2), :], (1, KP // 128))
                if half == 0:
                    w0, w1, w2 = [pltpu.bitcast(v << 16, f32) for v in ws]
                else:
                    w0, w1, w2 = [pltpu.bitcast(v & jnp.int32(-65536), f32) for v in ws]
                s = w0 + w2
                c6 = sT * (-1.0 / 6)
                p = w0 + 4.0 * w2
                q = w1 + w1
                c24 = sT * (1.0 / 24)
                res.append([w0 * (sT * 0.25), (s + w1) * c6, (s - w1) * c6, (p + q) * c24, (p - q) * c24, w2 * sT])
            for i in range(6):
                u_ref[i, pl.ds(r8, 8), :] = pltpu.bitcast(pltpu.pack_elementwise([res[0][i], res[1][i]], packed_dtype=bf16), i32)
            return carry
        jax.lax.fori_loop(0, C // 16, prep, 0, unroll=PU)

        def block(k, slot):
            b, t = k // TB, k % TB
            for n in range(NB):
                rows = [xs[b % 2, 4 * (NB * t + n) + j].astype(f32) for j in range(6)]
                d0, d1, d2, d3, d4, d5 = rows
                a = d4 - 4.0 * d2
                bb = d3 - 4.0 * d1
                c = d4 - d2
                e = 2.0 * (d3 - d1)
                vs = [4.0 * (d0 - d2) + c, a + bb, a - bb, c + e, c - e, (d5 - d3) - 2.0 * e]
                m = []
                for i in range(6):
                    u = pltpu.bitcast(u_ref[i], bf16)
                    v = vs[i].astype(bf16)
                    if KP != C:
                        v = jnp.concatenate([v, jnp.zeros((KP - C, BN), bf16)], axis=0)
                    m.append(jnp.dot(u, v, preferred_element_type=f32))
                m0, m1, m2, m3, m4, m5 = m
                m1 = m1 + jnp.tile(bias_ref[...], (1, BN // 128))
                s1 = m1 + m2; dd1 = m1 - m2; s2 = m3 + m4; dd2 = m3 - m4
                ys = [m0 + s1 + s2, dd1 + 2.0 * dd2, s1 + 4.0 * s2, dd1 + 8.0 * dd2 + m5]
                for j in range(4):
                    h = ys[j]
                    ob[n][slot, j] = (h * jnp.tanh(h) + h).astype(bf16)
                o_copy(k * NB + n, n, slot).start()

        x_copy(0).wait()

        def body(k, carry):
            for n in range(NB):
                @pl.when(k * NB + n + 1 < NU)
                def _():
                    x_copy(k * NB + n + 1).wait()
            for n in range(NB):
                @pl.when((k + 1) * NB + n + 1 < NU)
                def _():
                    x_copy((k + 1) * NB + n + 1).start()
            @pl.when(k >= 2)
            def _():
                for n in range(NB):
                    o_copy((k - 2) * NB + n, n, k % 2).wait()
            block(k, k % 2)
            return carry

        jax.lax.fori_loop(0, NBLK, body, 0)
        for k in range(NBLK - 2, NBLK):
            for n in range(NB):
                o_copy(k * NB + n, n, k % 2).wait()

    def fn(x, w, mean, var, g, b):
        B, S, C = x.shape
        xt = jnp.transpose(x, (1, 2, 0))
        vm = pl.BlockSpec(memory_space=pltpu.VMEM)
        out = pl.pallas_call(
            kernel,
            in_specs=[pl.BlockSpec(memory_space=pl.ANY), pl.BlockSpec(memory_space=pl.ANY), vm, vm, vm, vm],
            out_specs=pl.BlockSpec(memory_space=pl.ANY),
            out_shape=jax.ShapeDtypeStruct((S, C, B), x.dtype),
            scratch_shapes=[pltpu.VMEM((2, S + 2, C, BN), bf16), pltpu.VMEM((3, C, C), bf16), pltpu.SemaphoreType.DMA(()),
                            pltpu.VMEM((6, C // 2, KP), i32),
                            pltpu.VMEM((C, 128), f32), pltpu.VMEM((C, 128), f32), pltpu.VMEM((3, C // 2, KP), i32),
                            pltpu.SemaphoreType.DMA((2 * NB + 1,)), pltpu.SemaphoreType.DMA((2, NB))] + [pltpu.VMEM((2, 4, C, BN), bf16) for _ in range(NB)],
            compiler_params=pltpu.CompilerParams(vmem_limit_bytes=vmem * 2**20, flags=flags),
        )(xt, w, mean, var, g, b)
        return jnp.transpose(out, (2, 0, 1))
    return fn


@jax.jit
def pallas_standalone__batchnorm__sampling_kernel(x, w, mean, var, g, b):
    return _make()(x, w, mean, var, g, b)
```
